```python
import jax
import jax.numpy as jnp

def _softmax(x, axis=-1):
    return jax.nn.softmax(x, axis=axis)
def _gelu(x):
    return jax.nn.gelu(x, approximate=True)
def _silu(x):
    return jax.nn.silu(x)
def _sigmoid(x):
    return jax.nn.sigmoid(x)
def _layernorm(x, axis=-1, eps=1e-5):
    m = jnp.mean(x, axis=axis, keepdims=True)
    v = jnp.var(x, axis=axis, keepdims=True)
    return (x - m) / jnp.sqrt(v + eps)
def _scatter_add(tgt, idx, src, axis=0):
    return tgt.at[idx].add(src)
def _segment_sum(src, seg, n):
    return jax.ops.segment_sum(src, seg, n)
class _Rng:
    def __init__(self, key):
        self._k = key
    def _next(self):
        self._k, sub = jax.random.split(self._k)
        return sub
    def normal(self, shape):
        return jax.random.normal(self._next(), shape, dtype=jnp.bfloat16)
    def randint(self, lo, hi, shape):
        return jax.random.randint(self._next(), shape, lo, hi, dtype=jnp.int32)
    def uniform(self, shape, lo=0.0, hi=1.0):
        return jax.random.uniform(self._next(), shape, jnp.bfloat16, lo, hi)
    def permutation(self, n):
        return jax.random.permutation(self._next(), n)


kernel_name = 'gated_mix__compressed_kv_cla__gqa_block_cached__decode'

def setup_inputs():
    _rng = _Rng(jax.random.key(int.from_bytes(__import__("os").urandom(4), "little")))
    _w = (lambda a: (lambda t: t.astype(jnp.bfloat16) if jnp.issubdtype(t.dtype, jnp.floating) else t)(jnp.asarray(a)))
    def _A_setup():
        B, H, Sq, Sk, D, M = 1, 32, 1, 4096, 128, 640
        Dc = 4 * D
        return {
            "x": _w((lambda *s: _rng.normal(s) * 0.05)(B, Sq, M)),
            "c_kv": _w((lambda *s: _rng.normal(s) * 0.05)(B, Sk, Dc)),
            "w_q": _w((lambda *s: _rng.normal(s) * 0.05)(M, H, D) * (M ** -0.5)),
            "w_uk": _w((lambda *s: _rng.normal(s) * 0.05)(Dc, H, D) * (Dc ** -0.5)),
            "w_uv": _w((lambda *s: _rng.normal(s) * 0.05)(Dc, H, D) * (Dc ** -0.5)),
            "w_o": _w((lambda *s: _rng.normal(s) * 0.05)(H, D, M) * ((H * D) ** -0.5)),
        }
    _A_in = _A_setup()

    def _B_setup():
        B, Sq, D = 1, 1, 640
        Hq, Hkv, Sk, Dh = 32, 32, 4096, 128
        assert Hq % Hkv == 0, (Hq, Hkv)
        return {
            "x": _w((lambda *s: _rng.normal(s) * 0.05)(B, Sq, D)),
            "k_cache": _w((lambda *s: _rng.normal(s) * 0.05)(B, Hkv, Sk, Dh)),
            "v_cache": _w((lambda *s: _rng.normal(s) * 0.05)(B, Hkv, Sk, Dh)),
            "wq": _w((lambda *s: _rng.normal(s) * 0.05)(D, Hq * Dh) * (D ** -0.5)),
            "wo": _w((lambda *s: _rng.normal(s) * 0.05)(Hq * Dh, D) * ((Hq * Dh) ** -0.5)),
        }
    _B_in = _B_setup()

    return {
        "A_x": _A_in["x"],
        "A_c_kv": _A_in["c_kv"],
        "A_w_q": _A_in["w_q"],
        "A_w_uk": _A_in["w_uk"],
        "A_w_uv": _A_in["w_uv"],
        "A_w_o": _A_in["w_o"],
        "B_x": _B_in["x"],
        "B_k_cache": _B_in["k_cache"],
        "B_v_cache": _B_in["v_cache"],
        "B_wq": _B_in["wq"],
        "B_wo": _B_in["wo"],
        "gate_w": _w((lambda *s: _rng.normal(s) * 0.05)(640)),
    }

def reference(A_x, A_c_kv, A_w_q, A_w_uk, A_w_uv, A_w_o, B_x, B_k_cache, B_v_cache, B_wq, B_wo, gate_w):
    def _A_ref(x, c_kv, w_q, w_uk, w_uv, w_o):
        B, Sq, M = x.shape[0], x.shape[1], x.shape[2]
        Sk = c_kv.shape[1]
        H, D = w_q.shape[1], w_q.shape[2]
        q = jnp.einsum("bqm,mhd->bhqd", x, w_q)
        k = jnp.einsum("bkc,chd->bhkd", c_kv, w_uk)
        v = jnp.einsum("bkc,chd->bhkd", c_kv, w_uv)
        scores = jnp.einsum("bhqd,bhkd->bhqk", q, k) * (D ** -0.5)
        off = Sk - Sq
        qi = jnp.arange(Sq)[:, None]
        kj = jnp.arange(Sk)[None, :]
        cmask = kj <= (qi + off)
        scores = jnp.where(cmask[None, None], scores, -1e9)
        p = _softmax(scores, axis=-1)
        ctx = jnp.einsum("bhqk,bhkd->bhqd", p, v)
        return jnp.einsum("bhqd,hdm->bqm", ctx, w_o)

    def _B_ref(x, k_cache, v_cache, wq, wo):
        B, Sq, D = x.shape
        Hq, Dh = 32, 128
        Hkv = k_cache.shape[1]
        rep = Hq // Hkv
        q = (lambda x, *d: x.transpose(*d))((x @ wq).reshape(B, Sq, Hq, Dh), 0, 2, 1, 3)
        k = jnp.repeat(k_cache, rep, axis=1)
        v = jnp.repeat(v_cache, rep, axis=1)
        scores = jnp.einsum("bhqd,bhkd->bhqk", q, k) * (Dh ** -0.5)
        p = _softmax(scores, axis=-1)
        o = jnp.einsum("bhqk,bhkd->bhqd", p, v)
        return (lambda x, *d: x.transpose(*d))(o, 0, 2, 1, 3).reshape(B, Sq, Hq * Dh) @ wo

    x = A_x
    g = _sigmoid((x * gate_w).sum(-1, keepdims=True))
    a = _A_ref(x, A_c_kv, A_w_q, A_w_uk, A_w_uv, A_w_o)
    b = _B_ref(x, B_k_cache, B_v_cache, B_wq, B_wo)
    return g * a + (1 - g) * b
```

```python
import functools

import jax
import jax.numpy as jnp
import jax.experimental.pallas as pl
import jax.experimental.pallas.tpu as pltpu

H = 32
D = 128
S = 4096
M = 640
DC = 512
F32 = jnp.float32
BF16 = jnp.bfloat16

NT = (((1,), (1,)), ((), ()))


def _dot(a, b):
    return jnp.dot(a, b, preferred_element_type=F32)


def _dot_nt(a, b):
    return jax.lax.dot_general(a, b, NT, preferred_element_type=F32)


def _kernel(x_ref, gate_ref,
            ckv_hbm, awq_hbm, wuk_hbm, wuv_hbm, awo_hbm, k_hbm, v_hbm, bwq_hbm, bwo_hbm,
            out_ref,
            awq_buf, wuk_buf, ckv_buf, wuv_buf, awo_buf, bwq_buf, bwo_buf, k_buf, v_buf,
            rall_ref, qb_ref, wsem, ksem, vsem, *, HC):
    scale = D ** -0.5
    NCH = H // HC

    w_copies = [
        pltpu.make_async_copy(awq_hbm, awq_buf, wsem.at[0]),
        pltpu.make_async_copy(wuk_hbm, wuk_buf, wsem.at[1]),
        pltpu.make_async_copy(ckv_hbm.at[0], ckv_buf, wsem.at[2]),
        pltpu.make_async_copy(wuv_hbm, wuv_buf, wsem.at[3]),
        pltpu.make_async_copy(awo_hbm, awo_buf, wsem.at[4]),
        pltpu.make_async_copy(bwq_hbm, bwq_buf, wsem.at[5]),
        pltpu.make_async_copy(bwo_hbm, bwo_buf, wsem.at[6]),
    ]

    def k_copy(c):
        return pltpu.make_async_copy(k_hbm.at[0, pl.ds(c * HC, HC)],
                                     k_buf.at[pl.ds(c * HC, HC)], ksem.at[c])

    def v_copy(c):
        return pltpu.make_async_copy(v_hbm.at[0, pl.ds(c * HC, HC)],
                                     v_buf.at[pl.ds(c * HC, HC)], vsem.at[c])

    for cp in w_copies:
        cp.start()
    for c in range(NCH):
        k_copy(c).start()
        v_copy(c).start()

    r_row = jax.lax.broadcasted_iota(jnp.int32, (128, 4096), 0)
    r_col = jax.lax.broadcasted_iota(jnp.int32, (128, 4096), 1)
    rall_ref[...] = jnp.where(r_row == (r_col >> 5), 1.0, 0.0).astype(BF16)

    def diag_mask(rows):
        rr = jax.lax.broadcasted_iota(jnp.int32, (rows, 4096), 0)
        cc = jax.lax.broadcasted_iota(jnp.int32, (rows, 4096), 1)
        return (rr & 31) == (cc & 31)

    x = x_ref[0]
    xf = x.astype(F32)
    gw = gate_ref[...].reshape(1, M).astype(F32)
    g = jax.nn.sigmoid(jnp.sum(xf * gw, axis=-1, keepdims=True))

    def expand_contract(src_stack, w_buf, nk):
        e = _dot(src_stack, rall_ref[...])
        e = jnp.where(diag_mask(nk * 32), e, 0.0).astype(BF16)
        acc = jnp.zeros((H, D), F32)
        for kt in range(nk):
            w = w_buf[pl.ds(kt * 128, 128)].reshape(128 * H, D)
            acc = acc + _dot(e[kt * 32:(kt + 1) * 32], w)
        return acc

    xs = jnp.concatenate(
        [jnp.broadcast_to(x[:, kt * 128:(kt + 1) * 128], (H, 128)) for kt in range(M // 128)],
        axis=0)
    w_copies[0].wait()
    q_a = expand_contract(xs, awq_buf, M // 128).astype(BF16)

    w_copies[1].wait()
    m32 = diag_mask(H)
    pieces = []
    for kt in range(DC // 128):
        w = wuk_buf[pl.ds(kt * 128, 128)].reshape(128 * H, D)
        full = _dot_nt(q_a, w)
        pieces.append(jnp.where(m32, full, 0.0).astype(BF16))
    stack = jnp.concatenate(pieces, axis=0)
    qabs_stack = _dot_nt(stack, rall_ref[...]).astype(BF16)
    q_abs = jnp.concatenate([qabs_stack[kt * 32:(kt + 1) * 32] for kt in range(DC // 128)],
                            axis=1)

    w_copies[2].wait()
    ckv = ckv_buf[...]
    s = _dot_nt(q_abs, ckv) * scale
    m = jnp.max(s, axis=-1, keepdims=True)
    p = jnp.exp(s - m)
    l = jnp.sum(p, axis=-1, keepdims=True)
    lat = _dot(p.astype(BF16), ckv) / l
    lat_stack = jnp.concatenate([lat[:, kt * 128:(kt + 1) * 128] for kt in range(DC // 128)],
                                axis=0).astype(BF16)

    w_copies[3].wait()
    ctx = expand_contract(lat_stack, wuv_buf, DC // 128).astype(BF16)

    w_copies[4].wait()
    ctx_rep = jnp.concatenate([ctx] * H, axis=1)
    rr = jax.lax.broadcasted_iota(jnp.int32, (H, 4096), 0)
    cc = jax.lax.broadcasted_iota(jnp.int32, (H, 4096), 1)
    ctx_exp = jnp.where(rr == (cc >> 7), ctx_rep, jnp.zeros_like(ctx_rep))
    oa = _dot(ctx_exp, awo_buf[...].reshape(H * D, M))
    out_a = jnp.sum(oa, axis=0, keepdims=True)

    w_copies[5].wait()
    xb = jnp.broadcast_to(x, (8, M))
    qfull = _dot(xb, bwq_buf[...]).astype(BF16)
    for h in range(H):
        qb_ref[h] = qfull[:, h * D:(h + 1) * D]
    w_copies[6].wait()

    def chunk_body(c, acc):
        k_copy(c).wait()
        v_copy(c).wait()
        for j in range(HC):
            h = c * HC + j
            q = qb_ref[h]
            s = _dot_nt(q, k_buf[h]) * scale
            m = jnp.max(s, axis=-1, keepdims=True)
            p = jnp.exp(s - m)
            l = jnp.sum(p, axis=-1, keepdims=True)
            o = _dot(p.astype(BF16), v_buf[h]) / l
            wo = bwo_buf[pl.ds(pl.multiple_of(h * D, D), D), :]
            acc = acc + _dot(o.astype(BF16), wo)
        return acc

    acc = jax.lax.fori_loop(0, NCH, chunk_body, jnp.zeros((8, M), F32))
    out_b = acc[0:1]

    out = g * out_a + (1.0 - g) * out_b
    out_ref[0] = out.astype(out_ref.dtype)


@jax.jit
def pallas_gated_mix__compressed_kv_cla__gqa_block_cached__decode_kernel(
        A_x, A_c_kv, A_w_q, A_w_uk, A_w_uv, A_w_o, B_x, B_k_cache, B_v_cache, B_wq, B_wo, gate_w):
    HC = 4
    any_spec = pl.BlockSpec(memory_space=pl.ANY)
    vmem_spec = pl.BlockSpec(memory_space=pltpu.VMEM)
    if True:
        return pl.pallas_call(
            functools.partial(_kernel, HC=HC),
            out_shape=jax.ShapeDtypeStruct((1, 1, M), BF16),
            in_specs=[vmem_spec, vmem_spec] + [any_spec] * 9,
            out_specs=vmem_spec,
            scratch_shapes=[
                pltpu.VMEM((M, H, D), BF16),
                pltpu.VMEM((DC, H, D), BF16),
                pltpu.VMEM((S, DC), BF16),
                pltpu.VMEM((DC, H, D), BF16),
                pltpu.VMEM((H, D, M), BF16),
                pltpu.VMEM((M, H * D), BF16),
                pltpu.VMEM((H * D, M), BF16),
                pltpu.VMEM((H, S, D), BF16),
                pltpu.VMEM((H, S, D), BF16),
                pltpu.VMEM((128, 4096), BF16),
                pltpu.VMEM((H, 8, D), BF16),
                pltpu.SemaphoreType.DMA((7,)),
                pltpu.SemaphoreType.DMA((H // HC,)),
                pltpu.SemaphoreType.DMA((H // HC,)),
            ],
            compiler_params=pltpu.CompilerParams(vmem_limit_bytes=120 * 1024 * 1024),
        )(A_x, gate_w, A_c_kv, A_w_q, A_w_uk, A_w_uv, A_w_o, B_k_cache, B_v_cache, B_wq, B_wo)
```

```python
import functools

import jax
import jax.numpy as jnp
import jax.experimental.pallas as pl
import jax.experimental.pallas.tpu as pltpu

H = 32
D = 128
S = 4096
M = 640
DC = 512
F32 = jnp.float32
BF16 = jnp.bfloat16

KV_CHUNKS = (20, 9, 3)
WO_CHUNKS = (24, 6, 2)

_NT = (((1,), (1,)), ((), ()))


def _dot(a, b):
    return jnp.dot(a, b, preferred_element_type=F32)


def _dot_nt(a, b):
    return jax.lax.dot_general(a, b, _NT, preferred_element_type=F32)


def _starts(sizes):
    out, s = [], 0
    for n in sizes:
        out.append((s, n))
        s += n
    assert s == H
    return out


def _kernel(x_hbm, gate_hbm,
            ckv_hbm, awq_hbm, wuk_hbm, wuv_hbm, awo_hbm, k_hbm, v_hbm, bwq_hbm, bwo_hbm,
            out_ref,
            x_buf, g_buf,
            awq_buf, wuk_buf, ckv_buf, wuv_buf, awo_buf, bwq_buf, bwo_buf, k_buf, v_buf,
            rall_ref, qb_ref, ctxf_ref, acc_ref, sem):
    scale = D ** -0.5
    kv_chunks = _starts(KV_CHUNKS)
    wo_chunks = _starts(WO_CHUNKS)

    order = []

    def mk(src, dst):
        cp = pltpu.make_async_copy(src, dst, sem.at[len(order)])
        order.append(cp)
        return cp

    c_awq = mk(awq_hbm, awq_buf)
    c_x = mk(x_hbm, x_buf)
    c_g = mk(gate_hbm, g_buf)
    c_wuk = mk(wuk_hbm, wuk_buf)
    c_ckv = mk(ckv_hbm.at[0], ckv_buf)
    c_wuv = mk(wuv_hbm, wuv_buf)
    c_bwq = mk(bwq_hbm, bwq_buf)
    c_bwo = mk(bwo_hbm, bwo_buf)
    c_kv = []
    for (s0, n) in kv_chunks:
        ck = mk(k_hbm.at[0, pl.ds(s0, n)], k_buf.at[pl.ds(s0, n)])
        cv = mk(v_hbm.at[0, pl.ds(s0, n)], v_buf.at[pl.ds(s0, n)])
        c_kv.append((ck, cv))
    c_wo = [mk(awo_hbm.at[pl.ds(s0, n)], awo_buf.at[pl.ds(s0, n)]) for (s0, n) in wo_chunks]
    for cp in order:
        cp.start()

    r_row = jax.lax.broadcasted_iota(jnp.int32, (128, 4096), 0)
    r_col = jax.lax.broadcasted_iota(jnp.int32, (128, 4096), 1)
    rall_ref[...] = jnp.where(r_row == (r_col >> 5), 1.0, 0.0).astype(BF16)

    def diag_mask(rows):
        rr = jax.lax.broadcasted_iota(jnp.int32, (rows, 4096), 0)
        cc = jax.lax.broadcasted_iota(jnp.int32, (rows, 4096), 1)
        return (rr & 31) == (cc & 31)

    def expand_contract(src_stack, w_buf, nk):
        e = _dot(src_stack, rall_ref[...])
        e = jnp.where(diag_mask(nk * 32), e, 0.0).astype(BF16)
        acc = jnp.zeros((H, D), F32)
        for kt in range(nk):
            w = w_buf[pl.ds(kt * 128, 128)].reshape(128 * H, D)
            acc = acc + _dot(e[kt * 32:(kt + 1) * 32], w)
        return acc

    c_awq.wait()
    c_x.wait()
    c_g.wait()
    x = x_buf[0]
    xf = x.astype(F32)
    gwf = g_buf[...].reshape(1, M).astype(F32)
    g = jax.nn.sigmoid(jnp.sum(xf * gwf, axis=-1, keepdims=True))
    xs = jnp.concatenate(
        [jnp.broadcast_to(x[:, kt * 128:(kt + 1) * 128], (H, 128)) for kt in range(M // 128)],
        axis=0)
    q_a = expand_contract(xs, awq_buf, M // 128).astype(BF16)

    c_wuk.wait()
    m32 = diag_mask(H)
    pieces = []
    for kt in range(DC // 128):
        w = wuk_buf[pl.ds(kt * 128, 128)].reshape(128 * H, D)
        full = _dot_nt(q_a, w)
        pieces.append(jnp.where(m32, full, 0.0).astype(BF16))
    stack = jnp.concatenate(pieces, axis=0)
    qabs_stack = _dot_nt(stack, rall_ref[...]).astype(BF16)
    q_abs = jnp.concatenate([qabs_stack[kt * 32:(kt + 1) * 32] for kt in range(DC // 128)],
                            axis=1)

    c_ckv.wait()
    ckv = ckv_buf[...]
    s = _dot_nt(q_abs, ckv) * scale
    m = jnp.max(s, axis=-1, keepdims=True)
    p = jnp.exp(s - m)
    l = jnp.sum(p, axis=-1, keepdims=True)
    lat = _dot(p.astype(BF16), ckv) / l
    lat_stack = jnp.concatenate([lat[:, kt * 128:(kt + 1) * 128] for kt in range(DC // 128)],
                                axis=0).astype(BF16)

    c_wuv.wait()
    ctx = expand_contract(lat_stack, wuv_buf, DC // 128).astype(BF16)
    ctxf_ref[...] = jnp.concatenate(
        [jnp.broadcast_to(ctx[h:h + 1], (8, D)) for h in range(H)], axis=1)

    c_bwq.wait()
    xb = jnp.broadcast_to(x, (8, M))
    qfull = _dot(xb, bwq_buf[...]).astype(BF16)
    for h in range(H):
        qb_ref[h] = qfull[:, h * D:(h + 1) * D]
    c_bwo.wait()

    def head_body(h, acc):
        q = qb_ref[h]
        s = _dot_nt(q, k_buf[h]) * scale
        m = jnp.max(s, axis=-1, keepdims=True)
        p = jnp.exp(s - m)
        l = jnp.sum(p, axis=-1, keepdims=True)
        o = _dot(p.astype(BF16), v_buf[h]) / l
        wo = bwo_buf[pl.ds(pl.multiple_of(h * D, D), D), :]
        return acc + _dot(o.astype(BF16), wo)

    acc_b = jnp.zeros((8, M), F32)
    for (s0, n), (ck, cv) in zip(kv_chunks, c_kv):
        ck.wait()
        cv.wait()
        acc_b = jax.lax.fori_loop(s0, s0 + n, head_body, acc_b)

    acc_ref[...] = (1.0 - g) * acc_b
    npieces = len(wo_chunks)

    def tail_body(i, carry):
        for idx, ((s0, n), cw) in enumerate(zip(wo_chunks, c_wo)):
            @pl.when(i == idx)
            def _():
                cw.wait()
                d = _dot(ctxf_ref[:, s0 * D:(s0 + n) * D],
                         awo_buf[pl.ds(s0, n)].reshape(n * D, M))
                if idx == npieces - 1:
                    out_ref[0] = (acc_ref[0:1, :] + g * d[0:1]).astype(out_ref.dtype)
                else:
                    acc_ref[...] += g * d
        return carry

    jax.lax.fori_loop(0, npieces, tail_body, 0)


@jax.jit
def pallas_gated_mix__compressed_kv_cla__gqa_block_cached__decode_kernel(
    A_x: jax.Array,
    A_c_kv: jax.Array,
    A_w_q: jax.Array,
    A_w_uk: jax.Array,
    A_w_uv: jax.Array,
    A_w_o: jax.Array,
    B_x: jax.Array,
    B_k_cache: jax.Array,
    B_v_cache: jax.Array,
    B_wq: jax.Array,
    B_wo: jax.Array,
    gate_w: jax.Array,
):
    del B_x
    any_spec = pl.BlockSpec(memory_space=pl.ANY)
    nsem = 8 + 2 * len(KV_CHUNKS) + len(WO_CHUNKS)
    return pl.pallas_call(
        _kernel,
        out_shape=jax.ShapeDtypeStruct((1, 1, M), A_x.dtype),
        in_specs=[any_spec] * 11,
        out_specs=pl.BlockSpec(memory_space=pltpu.VMEM),
        scratch_shapes=[
            pltpu.VMEM((1, 1, M), BF16),
            pltpu.VMEM((M,), BF16),
            pltpu.VMEM((M, H, D), BF16),
            pltpu.VMEM((DC, H, D), BF16),
            pltpu.VMEM((S, DC), BF16),
            pltpu.VMEM((DC, H, D), BF16),
            pltpu.VMEM((H, D, M), BF16),
            pltpu.VMEM((M, H * D), BF16),
            pltpu.VMEM((H * D, M), BF16),
            pltpu.VMEM((H, S, D), BF16),
            pltpu.VMEM((H, S, D), BF16),
            pltpu.VMEM((128, 4096), BF16),
            pltpu.VMEM((H, 8, D), BF16),
            pltpu.VMEM((8, H * D), BF16),
            pltpu.VMEM((8, M), F32),
            pltpu.SemaphoreType.DMA((nsem,)),
        ],
        compiler_params=pltpu.CompilerParams(vmem_limit_bytes=120 * 1024 * 1024),
    )(A_x, gate_w, A_c_kv, A_w_q, A_w_uk, A_w_uv, A_w_o, B_k_cache, B_v_cache, B_wq, B_wo)
```

```python
import functools

import jax
import jax.numpy as jnp
import jax.experimental.pallas as pl
import jax.experimental.pallas.tpu as pltpu

H = 32
D = 128
S = 4096
M = 640
DC = 512
F32 = jnp.float32
BF16 = jnp.bfloat16

KV_CHUNKS = (20, 9, 3)
WO_CHUNKS = (24, 5, 2, 1)

_NT = (((1,), (1,)), ((), ()))


def _dot(a, b):
    return jnp.dot(a, b, preferred_element_type=F32)


def _dot_nt(a, b):
    return jax.lax.dot_general(a, b, _NT, preferred_element_type=F32)


def _starts(sizes):
    out, s = [], 0
    for n in sizes:
        out.append((s, n))
        s += n
    assert s == H
    return out


def _kernel(x_hbm, gate_hbm,
            ckv_hbm, awq_hbm, wuk_hbm, wuv_hbm, awo_hbm, k_hbm, v_hbm, bwq_hbm, bwo_hbm,
            out_ref,
            x_buf, g_buf,
            awq_buf, wuk_buf, ckv_buf, wuv_buf, awo_buf, bwq_buf, bwo_buf, k_buf, v_buf,
            rall_ref, qb_ref, ctxf_ref, acc_ref, sem):
    scale = D ** -0.5
    kv_chunks = _starts(KV_CHUNKS)
    wo_chunks = _starts(WO_CHUNKS)

    c_head = [pltpu.make_async_copy(src, dst, sem.at[0]) for src, dst in (
        (awq_hbm, awq_buf), (x_hbm, x_buf), (gate_hbm, g_buf), (wuk_hbm, wuk_buf),
        (ckv_hbm.at[0], ckv_buf), (wuv_hbm, wuv_buf), (bwq_hbm, bwq_buf), (bwo_hbm, bwo_buf))]
    c_kv = [(pltpu.make_async_copy(k_hbm.at[0, pl.ds(s0, n)], k_buf.at[pl.ds(s0, n)], sem.at[1 + i]),
             pltpu.make_async_copy(v_hbm.at[0, pl.ds(s0, n)], v_buf.at[pl.ds(s0, n)], sem.at[1 + i]))
            for i, (s0, n) in enumerate(kv_chunks)]
    c_wo = [pltpu.make_async_copy(awo_hbm.at[pl.ds(s0, n)], awo_buf.at[pl.ds(s0, n)],
                                  sem.at[1 + len(kv_chunks) + i])
            for i, (s0, n) in enumerate(wo_chunks)]
    for cp in c_head:
        cp.start()
    for ck, cv in c_kv:
        ck.start()
        cv.start()
    for cp in c_wo:
        cp.start()

    r_row = jax.lax.broadcasted_iota(jnp.int32, (128, 4096), 0)
    r_col = jax.lax.broadcasted_iota(jnp.int32, (128, 4096), 1)
    rall_ref[...] = jnp.where(r_row == (r_col >> 5), 1.0, 0.0).astype(BF16)

    def diag_mask(rows):
        rr = jax.lax.broadcasted_iota(jnp.int32, (rows, 4096), 0)
        cc = jax.lax.broadcasted_iota(jnp.int32, (rows, 4096), 1)
        return (rr & 31) == (cc & 31)

    def expand_contract(src_stack, w_buf, nk):
        e = _dot(src_stack, rall_ref[...])
        e = jnp.where(diag_mask(nk * 32), e, 0.0).astype(BF16)
        acc = jnp.zeros((H, D), F32)
        for kt in range(nk):
            w = w_buf[pl.ds(kt * 128, 128)].reshape(128 * H, D)
            acc = acc + _dot(e[kt * 32:(kt + 1) * 32], w)
        return acc

    for cp in c_head:
        cp.wait()

    x = x_buf[0]
    gwf = g_buf[...].reshape(1, M).astype(F32)
    g = jax.nn.sigmoid(jnp.sum(x.astype(F32) * gwf, axis=-1, keepdims=True))

    xs = jnp.concatenate(
        [jnp.broadcast_to(x[:, kt * 128:(kt + 1) * 128], (H, 128)) for kt in range(M // 128)],
        axis=0)
    q_a = expand_contract(xs, awq_buf, M // 128).astype(BF16)

    m32 = diag_mask(H)
    pieces = []
    for kt in range(DC // 128):
        w = wuk_buf[pl.ds(kt * 128, 128)].reshape(128 * H, D)
        full = _dot_nt(q_a, w)
        pieces.append(jnp.where(m32, full, 0.0).astype(BF16))
    stack = jnp.concatenate(pieces, axis=0)
    qabs_stack = _dot_nt(stack, rall_ref[...]).astype(BF16)
    q_abs = jnp.concatenate([qabs_stack[kt * 32:(kt + 1) * 32] for kt in range(DC // 128)],
                            axis=1)

    ckv = ckv_buf[...]
    s = _dot_nt(q_abs, ckv) * scale
    m = jnp.max(s, axis=-1, keepdims=True)
    p = jnp.exp(s - m)
    l = jnp.sum(p, axis=-1, keepdims=True)
    lat = _dot(p.astype(BF16), ckv) / l
    lat_stack = jnp.concatenate([lat[:, kt * 128:(kt + 1) * 128] for kt in range(DC // 128)],
                                axis=0).astype(BF16)

    ctx = expand_contract(lat_stack, wuv_buf, DC // 128).astype(BF16)
    ctxf_ref[...] = jnp.concatenate(
        [jnp.broadcast_to(ctx[h:h + 1], (8, D)) for h in range(H)], axis=1)

    qfull = _dot(jnp.broadcast_to(x, (8, M)), bwq_buf[...]).astype(BF16)
    for h in range(H):
        qb_ref[h] = qfull[:, h * D:(h + 1) * D]

    def head_body(h, acc):
        q = qb_ref[h]
        s = _dot_nt(q, k_buf[h]) * scale
        m = jnp.max(s, axis=-1, keepdims=True)
        p = jnp.exp(s - m)
        l = jnp.sum(p, axis=-1, keepdims=True)
        o = _dot(p.astype(BF16), v_buf[h]) / l
        wo = bwo_buf[pl.ds(pl.multiple_of(h * D, D), D), :]
        return acc + _dot(o.astype(BF16), wo)

    acc_b = jnp.zeros((8, M), F32)
    for (s0, n), (ck, cv) in zip(kv_chunks, c_kv):
        ck.wait()
        cv.wait()
        acc_b = jax.lax.fori_loop(s0, s0 + n, head_body, acc_b)

    acc_ref[...] = (1.0 - g) * acc_b
    last = len(wo_chunks) - 1

    def piece(idx):
        s0, n = wo_chunks[idx]
        c_wo[idx].wait()
        d = _dot(ctxf_ref[:, s0 * D:(s0 + n) * D], awo_buf[pl.ds(s0, n)].reshape(n * D, M))
        if idx == last:
            out_ref[0] = (acc_ref[0:1, :] + g * d[0:1]).astype(out_ref.dtype)
        else:
            acc_ref[...] += g * d

    def tail_body(i, carry):
        for idx in range(last):
            pl.when(i == idx)(functools.partial(piece, idx))
        return carry

    jax.lax.fori_loop(0, last, tail_body, 0)
    piece(last)


@jax.jit
def pallas_gated_mix__compressed_kv_cla__gqa_block_cached__decode_kernel(
    A_x: jax.Array,
    A_c_kv: jax.Array,
    A_w_q: jax.Array,
    A_w_uk: jax.Array,
    A_w_uv: jax.Array,
    A_w_o: jax.Array,
    B_x: jax.Array,
    B_k_cache: jax.Array,
    B_v_cache: jax.Array,
    B_wq: jax.Array,
    B_wo: jax.Array,
    gate_w: jax.Array,
):
    del B_x
    any_spec = pl.BlockSpec(memory_space=pl.ANY)
    return pl.pallas_call(
        _kernel,
        out_shape=jax.ShapeDtypeStruct((1, 1, M), A_x.dtype),
        in_specs=[any_spec] * 11,
        out_specs=pl.BlockSpec(memory_space=pltpu.VMEM),
        scratch_shapes=[
            pltpu.VMEM((1, 1, M), BF16),
            pltpu.VMEM((M,), BF16),
            pltpu.VMEM((M, H, D), BF16),
            pltpu.VMEM((DC, H, D), BF16),
            pltpu.VMEM((S, DC), BF16),
            pltpu.VMEM((DC, H, D), BF16),
            pltpu.VMEM((H, D, M), BF16),
            pltpu.VMEM((M, H * D), BF16),
            pltpu.VMEM((H * D, M), BF16),
            pltpu.VMEM((H, S, D), BF16),
            pltpu.VMEM((H, S, D), BF16),
            pltpu.VMEM((128, 4096), BF16),
            pltpu.VMEM((H, 8, D), BF16),
            pltpu.VMEM((8, H * D), BF16),
            pltpu.VMEM((8, M), F32),
            pltpu.SemaphoreType.DMA((1 + len(KV_CHUNKS) + len(WO_CHUNKS),)),
        ],
        compiler_params=pltpu.CompilerParams(vmem_limit_bytes=110 * 1024 * 1024),
    )(A_x, gate_w, A_c_kv, A_w_q, A_w_uk, A_w_uv, A_w_o, B_k_cache, B_v_cache, B_wq, B_wo)
```
